```python
import jax
import jax.numpy as jnp

def _softmax(x, axis=-1):
    return jax.nn.softmax(x, axis=axis)
def _gelu(x):
    return jax.nn.gelu(x, approximate=True)
def _silu(x):
    return jax.nn.silu(x)
def _sigmoid(x):
    return jax.nn.sigmoid(x)
def _layernorm(x, axis=-1, eps=1e-5):
    m = jnp.mean(x, axis=axis, keepdims=True)
    v = jnp.var(x, axis=axis, keepdims=True)
    return (x - m) / jnp.sqrt(v + eps)
def _scatter_add(tgt, idx, src, axis=0):
    return tgt.at[idx].add(src)
def _segment_sum(src, seg, n):
    return jax.ops.segment_sum(src, seg, n)
class _Rng:
    def __init__(self, key):
        self._k = key
    def _next(self):
        self._k, sub = jax.random.split(self._k)
        return sub
    def normal(self, shape):
        return jax.random.normal(self._next(), shape, dtype=jnp.bfloat16)
    def randint(self, lo, hi, shape):
        return jax.random.randint(self._next(), shape, lo, hi, dtype=jnp.int32)
    def uniform(self, shape, lo=0.0, hi=1.0):
        return jax.random.uniform(self._next(), shape, jnp.bfloat16, lo, hi)
    def permutation(self, n):
        return jax.random.permutation(self._next(), n)


kernel_name = 'parallel_sum__sliding_local_dilated__glu_gated_geglu__prompt'

def setup_inputs():
    _rng = _Rng(jax.random.key(int.from_bytes(__import__("os").urandom(4), "little")))
    _w = (lambda a: (lambda t: t.astype(jnp.bfloat16) if jnp.issubdtype(t.dtype, jnp.floating) else t)(jnp.asarray(a)))
    def _A_setup():
        B, S, D = 1, 2048, 1024
        return {
            "x": _w((lambda *s: _rng.normal(s) * 0.05)(B, S, D)),
            "wqkv": _w((lambda *s: _rng.normal(s) * 0.05)(D, 3 * D)),
            "wo": _w((lambda *s: _rng.normal(s) * 0.05)(D, D)),
        }
    _A_in = _A_setup()

    def _B_setup():
        B, S, Dm, Df = 1, 2048, 1024, 3584
        return {
            "x": _w((lambda *s: _rng.normal(s) * 0.05)(B, S, Dm)),
            "w_gate": _w((lambda *s: _rng.normal(s) * 0.05)(Dm, Df) * (Dm ** -0.5)),
            "w_up": _w((lambda *s: _rng.normal(s) * 0.05)(Dm, Df) * (Dm ** -0.5)),
            "w_down": _w((lambda *s: _rng.normal(s) * 0.05)(Df, Dm) * (Df ** -0.5)),
        }
    _B_in = _B_setup()

    return {
        "A_x": _A_in["x"],
        "A_wqkv": _A_in["wqkv"],
        "A_wo": _A_in["wo"],
        "B_x": _B_in["x"],
        "B_w_gate": _B_in["w_gate"],
        "B_w_up": _B_in["w_up"],
        "B_w_down": _B_in["w_down"],
    }

def reference(A_x, A_wqkv, A_wo, B_x, B_w_gate, B_w_up, B_w_down):
    def _A_ref(x, wqkv, wo):
        B, S, D = x.shape
        H = 32; Dh = D // H
        W, dil = 8, 2
        qkv = (lambda x, *d: x.transpose(*d))((x @ wqkv).reshape(B, S, 3, H, Dh), 2, 0, 3, 1, 4)
        q, k, v = qkv[0], qkv[1], qkv[2]
        scale = Dh ** -0.5
        pos = jnp.arange(S)
        off = jnp.arange(W) * dil
        idx = pos[:, None] - off[None, :]
        mask = idx >= 0
        idx_c = jnp.where(mask, idx, 0).reshape(-1)
        kg = k[:, :, idx_c, :].reshape(B, H, S, W, Dh)
        vg = v[:, :, idx_c, :].reshape(B, H, S, W, Dh)
        logits = jnp.einsum("bhsd,bhswd->bhsw", q, kg) * scale
        logits = jnp.where(mask[None, None, :, :], logits, -1e9)
        attn = _softmax(logits, axis=-1)
        o = jnp.einsum("bhsw,bhswd->bhsd", attn, vg)
        return (lambda x, *d: x.transpose(*d))(o, 0, 2, 1, 3).reshape(B, S, D) @ wo

    def _B_ref(x, w_gate, w_up, w_down):
        g = jnp.einsum("bsd,df->bsf", x, w_gate)
        u = jnp.einsum("bsd,df->bsf", x, w_up)
        h = _gelu(g) * u
        return jnp.einsum("bsf,fd->bsd", h, w_down)

    x = A_x
    xn = _layernorm(x, axis=-1)
    return x + _A_ref(xn, A_wqkv, A_wo) + _B_ref(xn, B_w_gate, B_w_up, B_w_down)
```

```python
import functools
import math

import jax
import jax.numpy as jnp
import numpy as np
from jax import lax
from jax.experimental import pallas as pl
from jax.experimental.pallas import tpu as pltpu

H = 32
W = 8
DIL = 2
HALO = 16
LANES = 128
F32 = jnp.float32
BF16 = jnp.bfloat16


def _layernorm(x):
  x = x.astype(F32)
  m = jnp.mean(x, axis=-1, keepdims=True)
  xc = x - m
  v = jnp.mean(xc * xc, axis=-1, keepdims=True)
  return (xc * lax.rsqrt(v + 1e-5)).astype(BF16)


def _gelu(x):
  c = math.sqrt(2.0 / math.pi)
  inner = x * (c + (c * 0.044715) * (x * x))
  hx = 0.5 * x
  return hx + hx * jnp.tanh(inner)


def _exchange(chunks):
  chunks = list(chunks)
  lane = lax.broadcasted_iota(jnp.int32, chunks[0].shape, 1)
  for b in range(3):
    s = 1 << b
    low = (lane & s) == 0
    for c in range(len(chunks)):
      if c & s:
        continue
      a, bb = chunks[c], chunks[c | s]
      chunks[c] = jnp.where(low, a, pltpu.roll(bb, s, 1))
      chunks[c | s] = jnp.where(low, pltpu.roll(a, LANES - s, 1), bb)
  return chunks


def make_kernel(T=256, FC=512, QC=512, RB=16, LB=16, peel=False, flags=None, wstep=1, ln_at="end", swp=True, ln_tick=True, NCH=256, per=None):
  def kernel(x_hbm, wqkv_hbm, wo_hbm, wg_hbm, wu_hbm, wd_hbm, o_ref,
             x_v, wqkv_v, wg_v, wu_v, w2_v, xn_v, qkv_v, h_v, sems, tok):
    S, D = x_hbm.shape
    F = wg_v.shape[1]
    NT = S // T
    NC = D // LANES
    nq = 3 * D // QC
    nf = F // FC
    i = pl.program_id(0)
    scale = (D // H) ** -0.5

    copies = {}
    n = 0

    def add(name, src, dst):
      nonlocal n
      copies[name] = pltpu.make_async_copy(src, dst, sems.at[n])
      n += 1

    add("x0", x_hbm.at[pl.ds(0, T)], x_v.at[pl.ds(0, T)])
    for j in range(nq):
      add(("q", j), wqkv_hbm.at[:, pl.ds(j * QC, QC)], wqkv_v.at[:, pl.ds(j * QC, QC)])
    for j in range(nf):
      add(("g", j), wg_hbm.at[:, pl.ds(j * FC, FC)], wg_v.at[:, pl.ds(j * FC, FC)])
      add(("u", j), wu_hbm.at[:, pl.ds(j * FC, FC)], wu_v.at[:, pl.ds(j * FC, FC)])
    add("x1", x_hbm.at[pl.ds(T, T)], x_v.at[pl.ds(T, T)])
    for j in range(D // NCH):
      cols = pl.ds(j * NCH, NCH)
      add(("d", j), wd_hbm.at[:, cols], w2_v.at[pl.ds(0, F), cols])
      add(("o", j), wo_hbm.at[:, cols], w2_v.at[pl.ds(F, D), cols])
    add("x2", x_hbm.at[pl.ds(2 * T, S - 2 * T)], x_v.at[pl.ds(2 * T, S - 2 * T)])

    chain = {}

    def after(val):
      prev = chain.get("prev")
      return val if prev is None else jnp.where(chain["true"], val, prev)

    def scores(r0):
      accs = [None] * W
      for c in range(NC):
        qc = after(qkv_v[c, pl.ds(HALO + r0, RB), :])
        for w in range(W):
          p = qc * qkv_v[NC + c, pl.ds(HALO + r0 - DIL * w, RB), :]
          accs[w] = p if accs[w] is None else accs[w] + p
        chain["prev"] = accs[W - 1]
      logits = []
      for w in range(W):
        acc = accs[w]
        acc = acc + pltpu.roll(acc, 8, 1)
        acc = acc + pltpu.roll(acc, 16, 1)
        if r0 < DIL * w:
          pos = i * T + r0 + lax.broadcasted_iota(jnp.int32, acc.shape, 0)
          acc = jnp.where(pos >= DIL * w, acc, -1e9)
        logits.append(acc)
      m = functools.reduce(jnp.maximum, logits)
      e = [jnp.exp(l - m) for l in logits]
      inv = 1.0 / functools.reduce(jnp.add, e)
      lane = lax.broadcasted_iota(jnp.int32, m.shape, 1)
      b16 = (lane & 16) != 0
      b8 = (lane & 8) != 0
      ps = []
      for w in range(W):
        p = e[w] * inv
        p = jnp.where(b16, p, pltpu.roll(p, LANES - 16, 1))
        ps.append(jnp.where(b8, p, pltpu.roll(p, LANES - 8, 1)))
      return ps

    def mix(r0, ps):
      o = [None] * NC
      for w in range(W):
        off = HALO + r0 - DIL * w
        pw = after(ps[w])
        for c in range(NC):
          t = pw * qkv_v[2 * NC + c, pl.ds(off, RB), :]
          o[c] = t if o[c] is None else o[c] + t
        chain["prev"] = o[NC - 1]
      o = _exchange(o)
      h_v[pl.ds(r0, RB), pl.ds(F, D)] = jnp.concatenate(o, axis=1).astype(BF16)

    def body(first):
      wait = (lambda name: copies[name].wait()) if first is True else (
          (lambda name: None) if first is False else
          (lambda name: pl.when(i == 0)(lambda: copies[name].wait())))
      slot = lax.rem(i, 2)
      chain.clear()
      chain['true'] = jnp.full((RB, LANES), tok[0], jnp.int32) == 0
      xn = xn_v.at[slot]

      def ln_next():
        wait("x1")
        nxt = jnp.minimum(i + 1, NT - 1)
        for r in range(0, T, LB):
          y = _layernorm(x_v[pl.ds(pl.multiple_of(nxt * T + r, LB), LB), :])
          xn_v[1 - slot, pl.ds(r, LB), :] = y

      if ln_at == "start":
        ln_next()
      for part in range(3):
        chunks = []
        for j in range(D // QC):
          jj = part * (D // QC) + j
          wait(("q", jj))
          r = jnp.dot(xn[...], wqkv_v[:, pl.ds(jj * QC, QC)], preferred_element_type=F32)
          if part == 0:
            r = r * scale
          chunks += [r[:, c * LANES:(c + 1) * LANES] for c in range(QC // LANES)]
        chunks = _exchange(chunks)
        for c in range(NC):
          qkv_v[part * NC + c, pl.ds(HALO, T), :] = chunks[c]
          if part == 2:
            qkv_v[part * NC + c, pl.ds(0, HALO), :] = jnp.where(
                i == 0, jnp.broadcast_to(chunks[c][0:1], (HALO, LANES)),
                qkv_v[part * NC + c, pl.ds(0, HALO), :])
      nrb = T // RB
      def attention_steps():
        ps = scores(0)
        for rb in range(nrb):
          nps = scores((rb + 1) * RB) if rb + 1 < nrb else None
          mix(rb * RB, ps)
          ps = nps
          yield
        for c in range(NC, 3 * NC):
          qkv_v[c, pl.ds(0, HALO), :] = qkv_v[c, pl.ds(T, HALO), :]
        yield
      steps = attention_steps()
      for j in range(nf):
        wait(("g", j))
        wait(("u", j))
        g = jnp.dot(xn[...], wg_v[:, pl.ds(j * FC, FC)], preferred_element_type=F32)
        u = jnp.dot(xn[...], wu_v[:, pl.ds(j * FC, FC)], preferred_element_type=F32)
        for _ in range(per[j]):
          next(steps)
        h_v[:, pl.ds(j * FC, FC)] = (_gelu(g) * u).astype(BF16)
      for _ in steps:
        pass
      if ln_at == "end":
        if ln_tick:
          x_v[pl.ds(S, 16), pl.ds(0, LANES)] = u[0:16, 0:LANES].astype(BF16)
        ln_next()
      for j in range(D // NCH):
        cols = pl.ds(j * NCH, NCH)
        wait(("d", j))
        wait(("o", j))
        r = jnp.dot(h_v[...], w2_v[:, cols], preferred_element_type=F32)
        xr = x_v[pl.ds(pl.multiple_of(i * T, T), T), cols].astype(F32)
        o_ref[:, cols] = (xr + r).astype(o_ref.dtype)

    @pl.when(i == 0)
    def _():
      for cp in copies.values():
        cp.start()
      tok[0] = 0
      qkv_v[:, pl.ds(0, HALO), :] = jnp.zeros((3 * NC, HALO, LANES), F32)
      copies["x0"].wait()
      xn_v[0] = _layernorm(x_v[pl.ds(0, T), :])

    @pl.when(i == 1)
    def _():
      copies["x2"].wait()

    if peel == "nowait":
      @pl.when(i == 0)
      def _():
        for name, cp in copies.items():
          if name not in ("x0", "x2"):
            cp.wait()
      body(False)
    elif peel:
      pl.when(i == 0)(lambda: body(True))
      pl.when(i > 0)(lambda: body(False))
    else:
      body(None)

  def f(A_x, A_wqkv, A_wo, B_x, B_w_gate, B_w_up, B_w_down):
    del B_x
    B, S, D = A_x.shape
    F = B_w_gate.shape[1]
    x = A_x.reshape(S, D)
    nsem = 3 + 3 * D // QC + 2 * (F // FC) + 2 * (D // NCH)
    any_spec = pl.BlockSpec(memory_space=pl.ANY)
    out = pl.pallas_call(
        kernel,
        grid=(S // T,),
        in_specs=[any_spec] * 6,
        out_specs=pl.BlockSpec((T, D), lambda i: (i, 0)),
        out_shape=jax.ShapeDtypeStruct((S, D), A_x.dtype),
        scratch_shapes=[
            pltpu.VMEM((S + 16, D), BF16),
            pltpu.VMEM((D, 3 * D), BF16),
            pltpu.VMEM((D, F), BF16),
            pltpu.VMEM((D, F), BF16),
            pltpu.VMEM((F + D, D), BF16),
            pltpu.VMEM((2, T, D), BF16),
            pltpu.VMEM((3 * D // LANES, T + HALO, LANES), F32),
            pltpu.VMEM((T, F + D), BF16),
            pltpu.SemaphoreType.DMA((nsem,)),
            pltpu.SMEM((1,), jnp.int32),
        ],
        compiler_params=pltpu.CompilerParams(
            dimension_semantics=("arbitrary",),
            vmem_limit_bytes=110 * 1024 * 1024, flags=flags,
        ),
        name="fused",
    )(x, A_wqkv, A_wo, B_w_gate, B_w_up, B_w_down)
    return out.reshape(B, S, D)

  return f


_impl = make_kernel(T=256, RB=8, LB=32, per=[5, 5, 5, 5, 4, 4, 4], ln_tick=False, NCH=512,
                    flags={"XLA_TPU_RESCHEDULE_DMA_DONES": True})


@jax.jit
def pallas_parallel_sum__sliding_local_dilated__glu_gated_geglu__prompt_kernel(
    A_x, A_wqkv, A_wo, B_x, B_w_gate, B_w_up, B_w_down):
  return _impl(A_x, A_wqkv, A_wo, B_x, B_w_gate, B_w_up, B_w_down)
```

```python
import functools
import math

import jax
import jax.numpy as jnp
import numpy as np
from jax import lax
from jax.experimental import pallas as pl
from jax.experimental.pallas import tpu as pltpu

H = 32
W = 8
DIL = 2
HALO = 16
LANES = 128
F32 = jnp.float32
BF16 = jnp.bfloat16
U32 = jnp.uint32


def _layernorm(x):
  x = x.astype(F32)
  m = jnp.mean(x, axis=-1, keepdims=True)
  xc = x - m
  v = jnp.mean(xc * xc, axis=-1, keepdims=True)
  return (xc * lax.rsqrt(v + 1e-5)).astype(BF16)


def _gelu(x):
  c = math.sqrt(2.0 / math.pi)
  inner = x * (c + (c * 0.044715) * (x * x))
  hx = 0.5 * x
  return hx + hx * jnp.tanh(inner)


def _exchange(chunks):
  chunks = list(chunks)
  lane = lax.broadcasted_iota(jnp.int32, chunks[0].shape, 1)
  for b in range(3):
    s = 1 << b
    low = (lane & s) == 0
    for c in range(len(chunks)):
      if c & s:
        continue
      a, bb = chunks[c], chunks[c | s]
      chunks[c] = jnp.where(low, a, pltpu.roll(bb, s, 1))
      chunks[c | s] = jnp.where(low, pltpu.roll(a, LANES - s, 1), bb)
  return chunks


def make_kernel(T=256, T1=512, FC=512, C0=256, RB=8, LB=32, NCH=1024, flags=None, mode="mem",
                ln_tick=True, prep_ahead=2, split_o=False):
  def kernel(x_hbm, wqkv_hbm, wo_hbm, wg_hbm, wu_hbm, wd_hbm, o_ref,
             x_v, wqkv_v, wg_v, wu_v, w2_v, xn_v, qkv_all, qkv_v, h_v, sems, tok):
    S, D = x_hbm.shape
    F = wg_v.shape[1]
    NC = D // LANES
    NR = S // T1
    n0 = D // C0
    nf = F // FC
    i = pl.program_id(0)
    scale = (D // H) ** -0.5
    half = T1 // 2

    def x_copy(r0, n, s):
      return pltpu.make_async_copy(x_hbm.at[pl.ds(r0, n)], x_v.at[pl.ds(r0, n)], sems.at[s])

    def wq_copy(j):
      cols = pl.ds(pl.multiple_of(j * C0, C0), C0)
      return pltpu.make_async_copy(wqkv_hbm.at[:, cols], wqkv_v.at[0, :, cols], sems.at[NR + 1 + j])

    def wkv_copy(p):
      return pltpu.make_async_copy(wqkv_hbm.at[:, pl.ds(p * D, D)], wqkv_v.at[p], sems.at[NR + n0 + p])

    s0 = NR + n0 + 3
    rest = [
        pltpu.make_async_copy(wg_hbm, wg_v, sems.at[s0]),
        pltpu.make_async_copy(wu_hbm, wu_v, sems.at[s0 + 1]),
        pltpu.make_async_copy(wd_hbm, w2_v.at[pl.ds(0, F)], sems.at[s0 + 2]),
        pltpu.make_async_copy(wo_hbm, w2_v.at[pl.ds(F, D)], sems.at[s0 + 3]),
    ]

    def ln_rows(r0, n, tick):
      for r in range(0, n, LB):
        rows = pl.ds(pl.multiple_of(r0 + r, LB), LB)
        y = _layernorm(x_v[rows, :])
        xn_v[rows, :] = y
        if tick:
          x_v[pl.ds(S, 16), pl.ds(0, LANES)] = y[0:16, 0:LANES]

    @pl.when(i == 0)
    def _():
      x_copy(0, half, 0).start()
      x_copy(half, half, NR).start()
      for j in range(n0):
        wq_copy(j).start()
      wkv_copy(1).start()
      x_copy(T1, T1, 1).start()
      wkv_copy(2).start()
      for r in range(2, NR):
        x_copy(r * T1, T1, r).start()
      for cp in rest:
        cp.start()
      tok[0] = 0
      qkv_v[:, pl.ds(0, HALO), :] = jnp.zeros((3 * NC, HALO, LANES), F32)

      def first_ln(j, _):
        x_copy(0, half, j * NR).wait()
        ln_rows(j * half, half, False)
      lax.fori_loop(0, 2, first_ln, None)

      def first_q(j, _):
        wq_copy(j).wait()
        cols = pl.ds(pl.multiple_of(j * C0, C0), C0)
        r = jnp.dot(xn_v[pl.ds(0, T1), :], wqkv_v[0, :, cols], preferred_element_type=F32)
        qkv_all[0, pl.ds(0, half), cols] = pltpu.bitcast(r.astype(BF16), U32)
      lax.fori_loop(0, n0, first_q, None)

      def proj(it, _):
        r = it // 3
        p = it - 3 * r
        nxt = jnp.minimum(r + 1, NR - 1)

        @pl.when(it < 3)
        def _():
          wkv_copy(p).wait()

        @pl.when((it == 1) | ((p == 0) & (r < NR - 1)))
        def _():
          x_copy(0, T1, nxt).wait()

        rows = pl.ds(pl.multiple_of(r * T1, T1), T1)
        y = jnp.dot(xn_v[rows, :], wqkv_v[p], preferred_element_type=F32)
        qkv_all[p, pl.ds(pl.multiple_of(r * half, half), half), :] = pltpu.bitcast(y.astype(BF16), U32)
        ln_rows(nxt * T1 + jnp.maximum(p - 1, 0) * half, half, ln_tick)
      lax.fori_loop(1, 3 * NR, proj, None)
      for cp in rest:
        cp.wait()

    chain = {}
    tok_row = pl.multiple_of(tok[0], 8)
    if mode == "sel":
      chain["true"] = jnp.full((RB, LANES), tok[0], jnp.int32) == 0

    def after(val):
      prev = chain.get("prev")
      if mode != "sel" or prev is None:
        return val
      return jnp.where(chain["true"], val, prev)

    def tick(val):
      if mode == "mem":
        qkv_v[0, pl.ds(tok_row, 8), :] = val[0:8]
      chain["prev"] = val

    def prep(g):
      rows = pl.ds(pl.multiple_of(i * (T // 2) + 8 * g, 8), 8)
      for p in range(3):
        chunks = _exchange([qkv_all[p, rows, pl.ds(c * LANES, LANES)] for c in range(NC)])
        for c in range(NC):
          y = pltpu.bitcast(chunks[c], BF16).astype(F32)
          qkv_v[p * NC + c, pl.ds(HALO + 16 * g, 16), :] = y
          if p == 2 and g == 0:
            qkv_v[p * NC + c, pl.ds(0, HALO), :] = jnp.where(
                i == 0, jnp.broadcast_to(y[0:1], (HALO, LANES)), qkv_v[p * NC + c, pl.ds(0, HALO), :])

    def scores(r0):
      accs = [None] * W
      if mode == "sel":
        for c in range(NC):
          qc = after(qkv_v[c, pl.ds(HALO + r0, RB), :])
          for w in range(W):
            t = qc * qkv_v[NC + c, pl.ds(HALO + r0 - DIL * w, RB), :]
            accs[w] = t if accs[w] is None else accs[w] + t
          tick(accs[W - 1])
      else:
        q = [qkv_v[c, pl.ds(HALO + r0, RB), :] for c in range(NC)]
        for w in range(W):
          for c in range(NC):
            t = q[c] * qkv_v[NC + c, pl.ds(HALO + r0 - DIL * w, RB), :]
            accs[w] = t if accs[w] is None else accs[w] + t
          tick(accs[w])
      logits = []
      for w in range(W):
        acc = accs[w]
        acc = acc + pltpu.roll(acc, 8, 1)
        acc = (acc + pltpu.roll(acc, 16, 1)) * scale
        if r0 < DIL * w:
          pos = i * T + r0 + lax.broadcasted_iota(jnp.int32, acc.shape, 0)
          acc = jnp.where(pos >= DIL * w, acc, -1e9)
        logits.append(acc)
      m = functools.reduce(jnp.maximum, logits)
      e = [jnp.exp(l - m) for l in logits]
      inv = 1.0 / functools.reduce(jnp.add, e)
      lane = lax.broadcasted_iota(jnp.int32, m.shape, 1)
      b16 = (lane & 16) != 0
      b8 = (lane & 8) != 0
      ps = []
      for w in range(W):
        p = e[w] * inv
        p = jnp.where(b16, p, pltpu.roll(p, LANES - 16, 1))
        ps.append(jnp.where(b8, p, pltpu.roll(p, LANES - 8, 1)))
      return ps

    def mix(r0, ps):
      o = [None] * NC
      for w in range(W):
        pw = after(ps[w])
        for c in range(NC):
          t = pw * qkv_v[2 * NC + c, pl.ds(HALO + r0 - DIL * w, RB), :]
          o[c] = t if o[c] is None else o[c] + t
        tick(o[NC - 1])
      return o

    ng = T // 16
    per = 16 // RB
    for g in range(min(prep_ahead, ng)):
      prep(g)
    ps = scores(0)
    outs = []
    for rb in range(T // RB):
      if rb % per == 0 and rb // per + prep_ahead < ng:
        prep(rb // per + prep_ahead)
      nps = scores((rb + 1) * RB) if (rb + 1) * RB < T else None
      outs.append(mix(rb * RB, ps))
      ps = nps
      if len(outs) == per:
        g = rb // per
        packed = [
            pltpu.bitcast(jnp.concatenate([o[c] for o in outs], axis=0).astype(BF16), U32)
            for c in range(NC)
        ]
        packed = _exchange(packed)
        for c in range(NC):
          h_v[pl.ds(16 * g, 16), pl.ds(F + c * LANES, LANES)] = pltpu.bitcast(packed[c], BF16)
        outs = []
    for c in range(NC, 3 * NC):
      qkv_v[c, pl.ds(0, HALO), :] = qkv_v[c, pl.ds(T, HALO), :]

    rows = pl.ds(pl.multiple_of(i * T, T), T)
    for j in range(nf):
      cols = pl.ds(j * FC, FC)
      g = jnp.dot(xn_v[rows, :], wg_v[:, cols], preferred_element_type=F32)
      u = jnp.dot(xn_v[rows, :], wu_v[:, cols], preferred_element_type=F32)
      h_v[:, cols] = (_gelu(g) * u).astype(BF16)
    for j in range(D // NCH):
      cols = pl.ds(j * NCH, NCH)
      if split_o:
        r = jnp.dot(h_v[:, pl.ds(0, F)], w2_v[pl.ds(0, F), cols], preferred_element_type=F32)
        r += jnp.dot(h_v[:, pl.ds(F, D)], w2_v[pl.ds(F, D), cols], preferred_element_type=F32)
      else:
        r = jnp.dot(h_v[...], w2_v[:, cols], preferred_element_type=F32)
      o_ref[:, cols] = (x_v[rows, cols].astype(F32) + r).astype(o_ref.dtype)

  def f(A_x, A_wqkv, A_wo, B_x, B_w_gate, B_w_up, B_w_down):
    del B_x
    B, S, D = A_x.shape
    F = B_w_gate.shape[1]
    x = A_x.reshape(S, D)
    nsem = S // T1 + D // C0 + 7
    any_spec = pl.BlockSpec(memory_space=pl.ANY)
    out = pl.pallas_call(
        kernel,
        grid=(S // T,),
        in_specs=[any_spec] * 6,
        out_specs=pl.BlockSpec((T, D), lambda i: (i, 0)),
        out_shape=jax.ShapeDtypeStruct((S, D), A_x.dtype),
        scratch_shapes=[
            pltpu.VMEM((S + 16, D), BF16),
            pltpu.VMEM((3, D, D), BF16),
            pltpu.VMEM((D, F), BF16),
            pltpu.VMEM((D, F), BF16),
            pltpu.VMEM((F + D, D), BF16),
            pltpu.VMEM((S, D), BF16),
            pltpu.VMEM((3, S // 2, D), U32),
            pltpu.VMEM((3 * D // LANES, T + HALO, LANES), F32),
            pltpu.VMEM((T, F + D), BF16),
            pltpu.SemaphoreType.DMA((nsem,)),
            pltpu.SMEM((1,), jnp.int32),
        ],
        compiler_params=pltpu.CompilerParams(
            dimension_semantics=("arbitrary",),
            vmem_limit_bytes=110 * 1024 * 1024, flags=flags,
        ),
        name="fused",
    )(x, A_wqkv, A_wo, B_w_gate, B_w_up, B_w_down)
    return out.reshape(B, S, D)

  return f


_impl = make_kernel(mode="sel")


@jax.jit
def pallas_parallel_sum__sliding_local_dilated__glu_gated_geglu__prompt_kernel(
    A_x, A_wqkv, A_wo, B_x, B_w_gate, B_w_up, B_w_down):
  return _impl(A_x, A_wqkv, A_wo, B_x, B_w_gate, B_w_up, B_w_down)
```

```python
import functools
import math

import jax
import jax.numpy as jnp
from jax import lax
from jax.experimental import pallas as pl
from jax.experimental.pallas import tpu as pltpu

HEADS = 32
WINDOW = 8
DILATION = 2
HALO = 16
LANES = 128

PROJ_ROWS = 512
FIRST_COLS = 256
LN_ROWS = 32
TILE_ROWS = 256
FF_COLS = 896
OUT_COLS = 128
ATT_ROWS = 8

F32 = jnp.float32
BF16 = jnp.bfloat16
U32 = jnp.uint32


def _layernorm(x):
  x = x.astype(F32)
  xc = x - jnp.mean(x, axis=-1, keepdims=True)
  var = jnp.mean(xc * xc, axis=-1, keepdims=True)
  return (xc * lax.rsqrt(var + 1e-5)).astype(BF16)


def _gelu(x):
  c = math.sqrt(2.0 / math.pi)
  half_x = 0.5 * x
  return half_x + half_x * jnp.tanh(x * (c + (c * 0.044715) * (x * x)))


def _swap_chunk_and_lane_bits(chunks):
  chunks = list(chunks)
  lane = lax.broadcasted_iota(jnp.int32, chunks[0].shape, 1)
  for bit in (1, 2, 4):
    low = (lane & bit) == 0
    for c in range(len(chunks)):
      if c & bit == 0:
        a, b = chunks[c], chunks[c | bit]
        chunks[c] = jnp.where(low, a, pltpu.roll(b, bit, 1))
        chunks[c | bit] = jnp.where(low, pltpu.roll(a, LANES - bit, 1), b)
  return chunks


def _kernel(x_hbm, wqkv_hbm, wo_hbm, wg_hbm, wu_hbm, wd_hbm, out_hbm,
            out_v, x_v, wqkv_v, wg_v, wu_v, w2_v, xn_v, qkv_packed, qkv_v, h_v, sems, zero):
  seq, dim = x_hbm.shape
  ff = wg_v.shape[1]
  nc = dim // LANES
  n_proj = seq // PROJ_ROWS
  n_first = dim // FIRST_COLS
  half = PROJ_ROWS // 2
  scale = (dim // HEADS) ** -0.5

  def x_copy(start, size, sem):
    rows = pl.ds(pl.multiple_of(start, size), size)
    return pltpu.make_async_copy(x_hbm.at[rows], x_v.at[rows], sems.at[sem])

  def wq_copy(j):
    cols = pl.ds(pl.multiple_of(j * FIRST_COLS, FIRST_COLS), FIRST_COLS)
    return pltpu.make_async_copy(
        wqkv_hbm.at[:, cols], wqkv_v.at[0, :, cols], sems.at[n_proj + 1 + j])

  def wkv_copy(part):
    cols = pl.ds(pl.multiple_of(part * dim, dim), dim)
    return pltpu.make_async_copy(
        wqkv_hbm.at[:, cols], wqkv_v.at[part], sems.at[n_proj + n_first + part])

  w_sem = sems.at[n_proj + n_first + 3]
  out_sem = sems.at[n_proj + n_first + 4]
  late_weights = [
      pltpu.make_async_copy(wg_hbm, wg_v, w_sem),
      pltpu.make_async_copy(wu_hbm, wu_v, w_sem),
      pltpu.make_async_copy(wd_hbm, w2_v.at[pl.ds(0, ff)], w_sem),
      pltpu.make_async_copy(wo_hbm, w2_v.at[pl.ds(ff, dim)], w_sem),
  ]

  def normalise(start, throttle):
    for r in range(0, half, LN_ROWS):
      rows = pl.ds(pl.multiple_of(start + r, LN_ROWS), LN_ROWS)
      y = _layernorm(x_v[rows, :])
      xn_v[rows, :] = y
      if throttle:
        x_v[pl.ds(seq, 16), pl.ds(0, LANES)] = y[0:16, 0:LANES]

  x_copy(0, half, 0).start()
  x_copy(half, half, n_proj).start()
  for j in range(n_first):
    wq_copy(j).start()
  wkv_copy(1).start()
  x_copy(PROJ_ROWS, PROJ_ROWS, 1).start()
  wkv_copy(2).start()
  for r in range(2, n_proj):
    x_copy(r * PROJ_ROWS, PROJ_ROWS, r).start()
  for copy in late_weights:
    copy.start()
  zero[0] = 0
  qkv_v[:, pl.ds(0, HALO), :] = jnp.zeros((3 * nc, HALO, LANES), F32)

  def first_norm(j, _):
    x_copy(j * half, half, j * n_proj).wait()
    normalise(j * half, False)

  lax.fori_loop(0, 2, first_norm, None)

  def first_projection(j, _):
    wq_copy(j).wait()
    cols = pl.ds(pl.multiple_of(j * FIRST_COLS, FIRST_COLS), FIRST_COLS)
    y = jnp.dot(xn_v[pl.ds(0, PROJ_ROWS), :], wqkv_v[0, :, cols], preferred_element_type=F32)
    qkv_packed[0, pl.ds(0, half), cols] = pltpu.bitcast(y.astype(BF16), U32)

  lax.fori_loop(0, n_first, first_projection, None)

  def projection(step, carry):
    r, part = carry
    nxt = jnp.minimum(r + 1, n_proj - 1)

    @pl.when(r == 0)
    def _():
      wkv_copy(part).wait()

    @pl.when((step == 1) | ((part == 0) & (r < n_proj - 1)))
    def _():
      x_copy(nxt * PROJ_ROWS, PROJ_ROWS, nxt).wait()

    rows = pl.ds(pl.multiple_of(r * PROJ_ROWS, PROJ_ROWS), PROJ_ROWS)
    y = jnp.dot(xn_v[rows, :], wqkv_v[part], preferred_element_type=F32)
    qkv_packed[part, pl.ds(pl.multiple_of(r * half, half), half), :] = pltpu.bitcast(
        y.astype(BF16), U32)
    normalise(nxt * PROJ_ROWS + jnp.maximum(part - 1, 0) * half, True)
    return jnp.where(part == 2, r + 1, r), jnp.where(part == 2, 0, part + 1)

  lax.fori_loop(1, 3 * n_proj, projection, (jnp.int32(0), jnp.int32(1)))
  for copy in late_weights:
    copy.wait()

  def out_copy(i, j):
    rows = pl.ds(pl.multiple_of(i * TILE_ROWS, TILE_ROWS), TILE_ROWS)
    cols = pl.ds(j * OUT_COLS, OUT_COLS)
    return pltpu.make_async_copy(out_v.at[rows, cols], out_hbm.at[rows, cols], out_sem)

  def tile(i, _):
    always = jnp.full((ATT_ROWS, LANES), zero[0], jnp.int32) == 0
    last = []

    def after(value):
      return jnp.where(always, value, last[-1]) if last else value

    def unpack(g):
      rows = pl.ds(pl.multiple_of(i * (TILE_ROWS // 2) + 8 * g, 8), 8)
      for part in range(3):
        chunks = _swap_chunk_and_lane_bits(
            [qkv_packed[part, rows, pl.ds(c * LANES, LANES)] for c in range(nc)])
        for c in range(nc):
          y = pltpu.bitcast(chunks[c], BF16).astype(F32)
          qkv_v[part * nc + c, pl.ds(HALO + 16 * g, 16), :] = y
          if part == 2 and g == 0:
            qkv_v[part * nc + c, pl.ds(0, HALO), :] = jnp.where(
                i == 0, jnp.broadcast_to(y[0:1], (HALO, LANES)),
                qkv_v[part * nc + c, pl.ds(0, HALO), :])

    def window(chunk, r0, w):
      return qkv_v[chunk, pl.ds(HALO + r0 - DILATION * w, ATT_ROWS), :]

    def probabilities(r0):
      dots = [None] * WINDOW
      for c in range(nc):
        q = after(window(c, r0, 0))
        for w in range(WINDOW):
          t = q * window(nc + c, r0, w)
          dots[w] = t if dots[w] is None else dots[w] + t
        last.append(dots[WINDOW - 1])
      logits = []
      for w in range(WINDOW):
        s = dots[w] + pltpu.roll(dots[w], 8, 1)
        s = (s + pltpu.roll(s, 16, 1)) * scale
        if r0 < DILATION * w:
          pos = i * TILE_ROWS + r0 + lax.broadcasted_iota(jnp.int32, s.shape, 0)
          s = jnp.where(pos >= DILATION * w, s, -1e9)
        logits.append(s)
      top = functools.reduce(jnp.maximum, logits)
      exps = [jnp.exp(s - top) for s in logits]
      inv = 1.0 / functools.reduce(jnp.add, exps)
      lane = lax.broadcasted_iota(jnp.int32, top.shape, 1)
      bit3, bit4 = (lane & 8) != 0, (lane & 16) != 0
      probs = []
      for e in exps:
        p = e * inv
        p = jnp.where(bit4, p, pltpu.roll(p, LANES - 16, 1))
        probs.append(jnp.where(bit3, p, pltpu.roll(p, LANES - 8, 1)))
      return probs

    def mix(r0, probs):
      out = [None] * nc
      for w in range(WINDOW):
        p = after(probs[w])
        for c in range(nc):
          t = p * window(2 * nc + c, r0, w)
          out[c] = t if out[c] is None else out[c] + t
        last.append(out[nc - 1])
      return out

    groups = TILE_ROWS // 16
    unpack(0)
    unpack(1)
    probs = probabilities(0)
    for g in range(groups):
      if g + 2 < groups:
        unpack(g + 2)
      outs = []
      for r0 in range(16 * g, 16 * g + 16, ATT_ROWS):
        ahead = probabilities(r0 + ATT_ROWS) if r0 + ATT_ROWS < TILE_ROWS else None
        outs.append(mix(r0, probs))
        probs = ahead
      packed = _swap_chunk_and_lane_bits([
          pltpu.bitcast(jnp.concatenate([o[c] for o in outs], axis=0).astype(BF16), U32)
          for c in range(nc)])
      for c in range(nc):
        h_v[pl.ds(16 * g, 16), pl.ds(ff + c * LANES, LANES)] = pltpu.bitcast(packed[c], BF16)
    for c in range(nc, 3 * nc):
      qkv_v[c, pl.ds(0, HALO), :] = qkv_v[c, pl.ds(TILE_ROWS, HALO), :]

    rows = pl.ds(pl.multiple_of(i * TILE_ROWS, TILE_ROWS), TILE_ROWS)
    for j in range(ff // FF_COLS):
      cols = pl.ds(j * FF_COLS, FF_COLS)
      gate = jnp.dot(xn_v[rows, :], wg_v[:, cols], preferred_element_type=F32)
      up = jnp.dot(xn_v[rows, :], wu_v[:, cols], preferred_element_type=F32)
      h_v[:, cols] = (_gelu(gate) * up).astype(BF16)
    for j in range(dim // OUT_COLS):
      cols = pl.ds(j * OUT_COLS, OUT_COLS)
      y = jnp.dot(h_v[...], w2_v[:, cols], preferred_element_type=F32)
      out_v[rows, cols] = (x_v[rows, cols].astype(F32) + y).astype(out_v.dtype)
      out_copy(i, j).start()

  lax.fori_loop(0, seq // TILE_ROWS, tile, None)
  for i in range(seq // TILE_ROWS):
    for j in range(dim // OUT_COLS):
      out_copy(i, j).wait()


@jax.jit
def pallas_parallel_sum__sliding_local_dilated__glu_gated_geglu__prompt_kernel(
    A_x: jax.Array,
    A_wqkv: jax.Array,
    A_wo: jax.Array,
    B_x: jax.Array,
    B_w_gate: jax.Array,
    B_w_up: jax.Array,
    B_w_down: jax.Array,
):
  del B_x
  batch, seq, dim = A_x.shape
  ff = B_w_gate.shape[1]
  assert batch == 1 and dim == 8 * LANES and dim // HEADS == 32
  assert seq % PROJ_ROWS == 0 and ff % FF_COLS == 0
  hbm = pl.BlockSpec(memory_space=pl.ANY)
  out = pl.pallas_call(
      _kernel,
      in_specs=[hbm] * 6,
      out_specs=hbm,
      out_shape=jax.ShapeDtypeStruct((seq, dim), A_x.dtype),
      scratch_shapes=[
          pltpu.VMEM((seq, dim), A_x.dtype),
          pltpu.VMEM((seq + 16, dim), BF16),
          pltpu.VMEM((3, dim, dim), BF16),
          pltpu.VMEM((dim, ff), BF16),
          pltpu.VMEM((dim, ff), BF16),
          pltpu.VMEM((ff + dim, dim), BF16),
          pltpu.VMEM((seq, dim), BF16),
          pltpu.VMEM((3, seq // 2, dim), U32),
          pltpu.VMEM((3 * dim // LANES, HALO + TILE_ROWS, LANES), F32),
          pltpu.VMEM((TILE_ROWS, ff + dim), BF16),
          pltpu.SemaphoreType.DMA((seq // PROJ_ROWS + dim // FIRST_COLS + 5,)),
          pltpu.SMEM((1,), jnp.int32),
      ],
      compiler_params=pltpu.CompilerParams(vmem_limit_bytes=100 * 1024 * 1024),
      name="attn_geglu",
  )(A_x.reshape(seq, dim), A_wqkv, A_wo, B_w_gate, B_w_up, B_w_down)
  return out.reshape(batch, seq, dim)
```

```python
import functools
import math

import jax
import jax.numpy as jnp
from jax import lax
from jax.experimental import pallas as pl
from jax.experimental.pallas import tpu as pltpu

HEADS = 32
WINDOW = 8
DILATION = 2
HALO = 16
LANES = 128

PROJ_ROWS = 512
FIRST_COLS = 256
LN_ROWS = 16
TILE_ROWS = 256
FF_COLS = 896
OUT_COLS = 128
ATT_ROWS = 8

F32 = jnp.float32
BF16 = jnp.bfloat16
U32 = jnp.uint32


def _layernorm(x):
  x = x.astype(F32)
  xc = x - jnp.mean(x, axis=-1, keepdims=True)
  var = jnp.mean(xc * xc, axis=-1, keepdims=True)
  return (xc * lax.rsqrt(var + 1e-5)).astype(BF16)


def _gelu(x):
  c = math.sqrt(2.0 / math.pi)
  half_x = 0.5 * x
  return half_x + half_x * jnp.tanh(x * (c + (c * 0.044715) * (x * x)))


def _swap_chunk_and_lane_bits(chunks):
  chunks = list(chunks)
  lane = lax.broadcasted_iota(jnp.int32, chunks[0].shape, 1)
  for bit in (1, 2, 4):
    low = (lane & bit) == 0
    for c in range(len(chunks)):
      if c & bit == 0:
        a, b = chunks[c], chunks[c | bit]
        chunks[c] = jnp.where(low, a, pltpu.roll(b, bit, 1))
        chunks[c | bit] = jnp.where(low, pltpu.roll(a, LANES - bit, 1), b)
  return chunks


def _kernel(x_hbm, wqkv_hbm, wo_hbm, wg_hbm, wu_hbm, wd_hbm, out_hbm,
            out_v, x_v, wqkv_v, wg_v, wu_v, w2_v, xn_v, qkv_packed, qkv_v, h_v, sems, zero):
  seq, dim = x_hbm.shape
  ff = wg_v.shape[1]
  nc = dim // LANES
  n_proj = seq // PROJ_ROWS
  wide = 3 * dim // 2
  n_first = wide // FIRST_COLS
  half = PROJ_ROWS // 2
  scale = (dim // HEADS) ** -0.5

  def x_copy(start, size, sem):
    rows = pl.ds(pl.multiple_of(start, size), size)
    return pltpu.make_async_copy(x_hbm.at[rows], x_v.at[rows], sems.at[sem])

  def w0_copy(j):
    cols = pl.ds(pl.multiple_of(j * FIRST_COLS, FIRST_COLS), FIRST_COLS)
    return pltpu.make_async_copy(
        wqkv_hbm.at[:, cols], wqkv_v.at[0, :, cols], sems.at[n_proj + 2 + j])

  w1_copy = pltpu.make_async_copy(
      wqkv_hbm.at[:, pl.ds(wide, wide)], wqkv_v.at[1], sems.at[n_proj + n_first + 2])
  w_sem = sems.at[n_proj + n_first + 3]
  out_sem = sems.at[n_proj + n_first + 4]
  late_weights = [
      pltpu.make_async_copy(wg_hbm, wg_v, w_sem),
      pltpu.make_async_copy(wu_hbm, wu_v, w_sem),
      pltpu.make_async_copy(wd_hbm, w2_v.at[pl.ds(0, ff)], w_sem),
      pltpu.make_async_copy(wo_hbm, w2_v.at[pl.ds(ff, dim)], w_sem),
  ]

  def normalise(start, size, throttle):
    for r in range(0, size, LN_ROWS):
      rows = pl.ds(pl.multiple_of(start + r, LN_ROWS), LN_ROWS)
      y = _layernorm(x_v[rows, :])
      xn_v[rows, :] = y
      if throttle:
        x_v[pl.ds(seq, 16), pl.ds(0, LANES)] = y[0:16, 0:LANES]

  x_copy(0, half, 0).start()
  x_copy(half, half, n_proj).start()
  for j in range(n_first):
    w0_copy(j).start()
    if j == 1:
      x_copy(PROJ_ROWS, half, n_proj + 1).start()
  x_copy(PROJ_ROWS + half, half, 1).start()
  w1_copy.start()
  for r in range(2, n_proj):
    x_copy(r * PROJ_ROWS, PROJ_ROWS, r).start()
  for copy in late_weights:
    copy.start()
  zero[0] = 0
  qkv_v[:, pl.ds(0, HALO), :] = jnp.zeros((3 * nc, HALO, LANES), F32)

  def first_norm(j, _):
    x_copy(j * half, half, j * n_proj).wait()
    normalise(j * half, half, False)

  lax.fori_loop(0, 2, first_norm, None)

  def first_projection(j, _):
    w0_copy(j).wait()

    @pl.when(j == 2)
    def _():
      x_copy(PROJ_ROWS, half, n_proj + 1).wait()

    cols = pl.ds(pl.multiple_of(j * FIRST_COLS, FIRST_COLS), FIRST_COLS)
    y = jnp.dot(xn_v[pl.ds(0, PROJ_ROWS), :], wqkv_v[0, :, cols], preferred_element_type=F32)
    qkv_packed[0, pl.ds(0, half), cols] = pltpu.bitcast(y.astype(BF16), U32)
    size = half // (n_first - 2)
    normalise(PROJ_ROWS + (j - 2) * size, size, True)

  lax.fori_loop(0, n_first, first_projection, None)
  x_copy(PROJ_ROWS + half, half, 1).wait()
  w1_copy.wait()

  def projection(step, _):
    r, part = step >> 1, step & 1
    nxt = jnp.minimum(r + 1, n_proj - 1)

    @pl.when((part == 0) & (r < n_proj - 1))
    def _():
      x_copy(nxt * PROJ_ROWS, PROJ_ROWS, nxt).wait()

    rows = pl.ds(pl.multiple_of(r * PROJ_ROWS, PROJ_ROWS), PROJ_ROWS)
    y = jnp.dot(xn_v[rows, :], wqkv_v[part], preferred_element_type=F32)
    qkv_packed[part, pl.ds(pl.multiple_of(r * half, half), half), :] = pltpu.bitcast(
        y.astype(BF16), U32)
    normalise(nxt * PROJ_ROWS + part * half, half, True)

  lax.fori_loop(1, 2 * n_proj, projection, None)
  for copy in late_weights:
    copy.wait()

  def out_copy(i, j):
    rows = pl.ds(pl.multiple_of(i * TILE_ROWS, TILE_ROWS), TILE_ROWS)
    cols = pl.ds(j * OUT_COLS, OUT_COLS)
    return pltpu.make_async_copy(out_v.at[rows, cols], out_hbm.at[rows, cols], out_sem)

  def tile(i, _):
    always = jnp.full((ATT_ROWS, LANES), zero[0], jnp.int32) == 0
    last = []

    def after(value):
      return jnp.where(always, value, last[-1]) if last else value

    def unpack(g):
      rows = pl.ds(pl.multiple_of(i * (TILE_ROWS // 2) + 8 * g, 8), 8)
      for part in range(3):
        chunks = _swap_chunk_and_lane_bits(
            [qkv_packed[col // wide, rows, pl.ds(col % wide, LANES)]
             for col in range(part * dim, (part + 1) * dim, LANES)])
        for c in range(nc):
          y = pltpu.bitcast(chunks[c], BF16).astype(F32)
          qkv_v[part * nc + c, pl.ds(HALO + 16 * g, 16), :] = y
          if part == 2 and g == 0:
            qkv_v[part * nc + c, pl.ds(0, HALO), :] = jnp.where(
                i == 0, jnp.broadcast_to(y[0:1], (HALO, LANES)),
                qkv_v[part * nc + c, pl.ds(0, HALO), :])

    def window(chunk, r0, w):
      return qkv_v[chunk, pl.ds(HALO + r0 - DILATION * w, ATT_ROWS), :]

    def probabilities(r0):
      dots = [None] * WINDOW
      for c in range(nc):
        q = after(window(c, r0, 0))
        for w in range(WINDOW):
          t = q * window(nc + c, r0, w)
          dots[w] = t if dots[w] is None else dots[w] + t
        last.append(dots[WINDOW - 1])
      logits = []
      for w in range(WINDOW):
        s = dots[w] + pltpu.roll(dots[w], 8, 1)
        s = (s + pltpu.roll(s, 16, 1)) * scale
        if r0 < DILATION * w:
          pos = i * TILE_ROWS + r0 + lax.broadcasted_iota(jnp.int32, s.shape, 0)
          s = jnp.where(pos >= DILATION * w, s, -1e9)
        logits.append(s)
      top = functools.reduce(jnp.maximum, logits)
      exps = [jnp.exp(s - top) for s in logits]
      inv = 1.0 / functools.reduce(jnp.add, exps)
      lane = lax.broadcasted_iota(jnp.int32, top.shape, 1)
      bit3, bit4 = (lane & 8) != 0, (lane & 16) != 0
      probs = []
      for e in exps:
        p = e * inv
        p = jnp.where(bit4, p, pltpu.roll(p, LANES - 16, 1))
        probs.append(jnp.where(bit3, p, pltpu.roll(p, LANES - 8, 1)))
      return probs

    def mix(r0, probs):
      out = [None] * nc
      for w in range(WINDOW):
        p = after(probs[w])
        for c in range(nc):
          t = p * window(2 * nc + c, r0, w)
          out[c] = t if out[c] is None else out[c] + t
        last.append(out[nc - 1])
      return out

    groups = TILE_ROWS // 16
    unpack(0)
    unpack(1)
    probs = probabilities(0)
    for g in range(groups):
      if g + 2 < groups:
        unpack(g + 2)
      outs = []
      for r0 in range(16 * g, 16 * g + 16, ATT_ROWS):
        ahead = probabilities(r0 + ATT_ROWS) if r0 + ATT_ROWS < TILE_ROWS else None
        outs.append(mix(r0, probs))
        probs = ahead
      packed = _swap_chunk_and_lane_bits([
          pltpu.bitcast(jnp.concatenate([o[c] for o in outs], axis=0).astype(BF16), U32)
          for c in range(nc)])
      for c in range(nc):
        h_v[pl.ds(16 * g, 16), pl.ds(ff + c * LANES, LANES)] = pltpu.bitcast(packed[c], BF16)
    for c in range(nc, 3 * nc):
      qkv_v[c, pl.ds(0, HALO), :] = qkv_v[c, pl.ds(TILE_ROWS, HALO), :]

    rows = pl.ds(pl.multiple_of(i * TILE_ROWS, TILE_ROWS), TILE_ROWS)
    for j in range(ff // FF_COLS):
      cols = pl.ds(j * FF_COLS, FF_COLS)
      gate = jnp.dot(xn_v[rows, :], wg_v[:, cols], preferred_element_type=F32)
      up = jnp.dot(xn_v[rows, :], wu_v[:, cols], preferred_element_type=F32)
      h_v[:, cols] = (_gelu(gate) * up).astype(BF16)
    for j in range(dim // OUT_COLS):
      cols = pl.ds(j * OUT_COLS, OUT_COLS)
      y = jnp.dot(h_v[...], w2_v[:, cols], preferred_element_type=F32)
      out_v[rows, cols] = (x_v[rows, cols].astype(F32) + y).astype(out_v.dtype)
      out_copy(i, j).start()

  lax.fori_loop(0, seq // TILE_ROWS, tile, None)
  for i in range(seq // TILE_ROWS):
    for j in range(dim // OUT_COLS):
      out_copy(i, j).wait()


@jax.jit
def pallas_parallel_sum__sliding_local_dilated__glu_gated_geglu__prompt_kernel(
    A_x: jax.Array,
    A_wqkv: jax.Array,
    A_wo: jax.Array,
    B_x: jax.Array,
    B_w_gate: jax.Array,
    B_w_up: jax.Array,
    B_w_down: jax.Array,
):
  del B_x
  batch, seq, dim = A_x.shape
  ff = B_w_gate.shape[1]
  assert batch == 1 and dim == 8 * LANES and dim // HEADS == 32
  assert seq % PROJ_ROWS == 0 and ff % FF_COLS == 0
  hbm = pl.BlockSpec(memory_space=pl.ANY)
  out = pl.pallas_call(
      _kernel,
      in_specs=[hbm] * 6,
      out_specs=hbm,
      out_shape=jax.ShapeDtypeStruct((seq, dim), A_x.dtype),
      scratch_shapes=[
          pltpu.VMEM((seq, dim), A_x.dtype),
          pltpu.VMEM((seq + 16, dim), BF16),
          pltpu.VMEM((2, dim, 3 * dim // 2), BF16),
          pltpu.VMEM((dim, ff), BF16),
          pltpu.VMEM((dim, ff), BF16),
          pltpu.VMEM((ff + dim, dim), BF16),
          pltpu.VMEM((seq, dim), BF16),
          pltpu.VMEM((2, seq // 2, 3 * dim // 2), U32),
          pltpu.VMEM((3 * dim // LANES, HALO + TILE_ROWS, LANES), F32),
          pltpu.VMEM((TILE_ROWS, ff + dim), BF16),
          pltpu.SemaphoreType.DMA((seq // PROJ_ROWS + 3 * dim // 2 // FIRST_COLS + 5,)),
          pltpu.SMEM((1,), jnp.int32),
      ],
      compiler_params=pltpu.CompilerParams(vmem_limit_bytes=100 * 1024 * 1024),
      name="attn_geglu",
  )(A_x.reshape(seq, dim), A_wqkv, A_wo, B_w_gate, B_w_up, B_w_down)
  return out.reshape(batch, seq, dim)
```
